```python
import os as _os
_os.environ.setdefault("JAX_PLATFORMS", "cpu")
import jax
import jax.numpy as jnp

def _softmax(x, axis=-1):
    return jax.nn.softmax(x, axis=axis)
def _gelu(x):
    return jax.nn.gelu(x, approximate=True)
def _silu(x):
    return jax.nn.silu(x)
def _sigmoid(x):
    return jax.nn.sigmoid(x)
def _layernorm(x, axis=-1, eps=1e-5):
    m = jnp.mean(x, axis=axis, keepdims=True)
    v = jnp.var(x, axis=axis, keepdims=True)
    return (x - m) / jnp.sqrt(v + eps)
def _scatter_add(tgt, idx, src, axis=0):
    return tgt.at[idx].add(src)
def _segment_sum(src, seg, n):
    return jax.ops.segment_sum(src, seg, n)
class _Rng:
    def __init__(self, key):
        self._k = key
    def _next(self):
        self._k, sub = jax.random.split(self._k)
        return sub
    def normal(self, shape):
        return jax.random.normal(self._next(), shape, dtype=jnp.bfloat16)
    def randint(self, lo, hi, shape):
        return jax.random.randint(self._next(), shape, lo, hi, dtype=jnp.int32)
    def uniform(self, shape, lo=0.0, hi=1.0):
        return jax.random.uniform(self._next(), shape, jnp.bfloat16, lo, hi)
    def permutation(self, n):
        return jax.random.permutation(self._next(), n)


kernel_name = 'standalone__mha_block_cached__near_ridge'

def setup_inputs():
    _rng = _Rng(jax.random.key(int.from_bytes(__import__("os").urandom(4), "little")))
    _w = (lambda a: (lambda t: t.astype(jnp.bfloat16) if jnp.issubdtype(t.dtype, jnp.floating) else t)(jnp.asarray(a)))
    B, Sq, D = 8, 96, 576
    H, Sk, Dh = 32, 96, 128
    return {
        "x": _w((lambda *s: _rng.normal(s) * 0.8)(B, Sq, D)),
        "k_cache": _w((lambda *s: _rng.normal(s) * 0.8)(B, H, Sk, Dh)),
        "v_cache": _w((lambda *s: _rng.normal(s) * 0.05)(B, H, Sk, Dh)),
        "wq": _w((lambda *s: _rng.normal(s) * 0.8)(D, H * Dh) * (D ** -0.5)),
        "wo": _w((lambda *s: _rng.normal(s) * 0.05)(H * Dh, D) * ((H * Dh) ** -0.5)),
    }

def reference(x, k_cache, v_cache, wq, wo):
    B, Sq, D = x.shape
    H, Dh = 32, 128
    q = (lambda x, *d: x.transpose(*d))((x @ wq).reshape(B, Sq, H, Dh), 0, 2, 1, 3)
    scores = jnp.einsum("bhqd,bhkd->bhqk", q, k_cache) * (Dh ** -0.5)
    p = _softmax(scores, axis=-1)
    o = jnp.einsum("bhqk,bhkd->bhqd", p, v_cache)
    return (lambda x, *d: x.transpose(*d))(o, 0, 2, 1, 3).reshape(B, Sq, H * Dh) @ wo
```

```python
import functools
import math
import jax
import jax.numpy as jnp
import jax.experimental.pallas as pl
import jax.experimental.pallas.tpu as pltpu

HG = 4
KA = 256
NT = (((1,), (1,)), ((), ()))
f32, bf16 = jnp.float32, jnp.bfloat16


def _kernel(x_hbm, k_hbm, v_hbm, wq_hbm, wot_hbm, o_hbm,
            x_v, k_v, v_v, wq_v, wot_v, acc_ref, q_ref, ob_ref, out_v, qp_ref, sems,
            *, B, Sq, D, H, Dh, scale):
    G = H // HG
    W = HG * Dh
    RP = 2 * Sq
    NJ = (B * Sq) // 128
    S1, S2, S3, S4, SL, SO = range(6)

    def wq_cp(g, s):
        return pltpu.make_async_copy(wq_hbm.at[:, pl.ds(g * W, W)], wq_v.at[g], sems.at[s])

    def wot_cp(g, s):
        return pltpu.make_async_copy(wot_hbm.at[:, pl.ds(g * W, W)], wot_v.at[g], sems.at[s])

    def k_cp(g, s):
        return pltpu.make_async_copy(k_hbm.at[:, pl.ds(g * HG, HG)], k_v.at[g], sems.at[s])

    def v_cp(g, s):
        return pltpu.make_async_copy(v_hbm.at[:, pl.ds(g * HG, HG)], v_v.at[g], sems.at[s])

    def out_cp(j):
        return pltpu.make_async_copy(out_v.at[pl.ds(j * 128, 128)], o_hbm.at[pl.ds(j * 128, 128)], sems.at[SO])

    def grp1():
        return (pltpu.make_async_copy(x_hbm.at[:, pl.ds(0, KA)], x_v.at[:, pl.ds(0, KA)], sems.at[S1]),
                pltpu.make_async_copy(wq_hbm.at[pl.ds(0, KA), pl.ds(0, W)], wq_v.at[0, pl.ds(0, KA)], sems.at[S1]))

    def grp2():
        return (pltpu.make_async_copy(x_hbm.at[:, pl.ds(KA, D - KA)], x_v.at[:, pl.ds(KA, D - KA)], sems.at[S2]),
                pltpu.make_async_copy(wq_hbm.at[pl.ds(KA, D - KA), pl.ds(0, W)], wq_v.at[0, pl.ds(KA, D - KA)],
                                      sems.at[S2]))

    def grp3():
        return (k_cp(0, S3), wq_cp(1, S3))

    def grp4():
        return (v_cp(0, S4), wot_cp(0, S4))

    def kvo(g):
        return (k_cp(g, SL), v_cp(g, SL), wot_cp(g, SL))

    def start(cs, prio=1):
        for c in cs:
            c.start(priority=prio)

    def wait(cs):
        for c in cs:
            c.wait()

    def Q(g, bp):
        r = slice(bp * RP, (bp + 1) * RP)
        q_ref[r, :] = (jnp.dot(x_v[r, :], wq_v[g], preferred_element_type=f32) * scale).astype(bf16)

    def QK(g, bp):
        res = []
        for b in (2 * bp, 2 * bp + 1):
            for h in range(HG):
                qbh = q_ref[b * Sq:(b + 1) * Sq, h * Dh:(h + 1) * Dh]
                res.append((b, h, jax.lax.dot_general(qbh, k_v[g, b, h], NT, preferred_element_type=f32)))
        return res

    def SM(ss):
        res = []
        for b, h, s in ss:
            m = jnp.max(s, axis=-1, keepdims=True)
            p = jnp.exp2(s - m)
            l = jnp.sum(p, axis=-1, keepdims=True)
            res.append((b, h, p.astype(bf16), pl.reciprocal(l, approx=True)))
        return res

    def PV(g, ps):
        for b, h, p, r in ps:
            o = jnp.dot(p, v_v[g, b, h], preferred_element_type=f32)
            ob_ref[b * Sq:(b + 1) * Sq, h * Dh:(h + 1) * Dh] = (o * r).astype(bf16)

    def O(g, j, mode='acc'):
        c = slice(j * 128, (j + 1) * 128)
        part = jax.lax.dot_general(wot_v[g], ob_ref[c, :], NT, preferred_element_type=f32)
        if mode == 'set':
            acc_ref[:, c] = part
        elif mode == 'out':
            out_v[c, :] = (acc_ref[:, c] + part).T.astype(out_v.dtype)
            out_cp(j).start()
        else:
            acc_ref[:, c] += part

    start(grp1(), 0)
    start(grp2(), 1)
    acc_ref[:, 4 * 128:] = jnp.zeros((D, (NJ - 4) * 128), f32)
    wait(grp1())
    start(grp3())
    qp_ref[...] = jnp.dot(x_v[:, :KA], wq_v[0, :KA, :], preferred_element_type=f32)
    wait(grp2())
    start(grp4())
    q_ref[...] = ((qp_ref[...] + jnp.dot(x_v[:, KA:], wq_v[0, KA:, :], preferred_element_type=f32)) * scale).astype(bf16)
    wait(grp3())
    start(kvo(1) + (wq_cp(2, SL),))
    s0 = QK(0, 0); Q(1, 0); p0 = SM(s0); s1 = QK(0, 1); Q(1, 1); p1 = SM(s1); s2 = QK(0, 2); Q(1, 2); p2 = SM(s2)
    wait(grp4())
    s3 = QK(0, 3); PV(0, p0); PV(0, p1); PV(0, p2); Q(1, 3); PV(0, SM(s3))
    for j in range(4):
        O(0, j, 'set')

    def body(g, carry):
        wait(kvo(g) + (wq_cp(g + 1, SL),))
        start(kvo(g + 1))

        @pl.when(g + 2 < G)
        def _():
            start((wq_cp(g + 2, SL),))

        s0 = QK(g, 0); O(g - 1, 4); PV(g, SM(s0)); s1 = QK(g, 1); O(g - 1, 5); Q(g + 1, 0); PV(g, SM(s1))
        s2 = QK(g, 2); O(g, 0); Q(g + 1, 1); PV(g, SM(s2)); s3 = QK(g, 3)
        O(g, 1); O(g, 2); Q(g + 1, 2); PV(g, SM(s3)); Q(g + 1, 3); O(g, 3)
        return carry

    jax.lax.fori_loop(1, G - 1, body, 0)

    g = G - 1
    wait(kvo(g))
    s0 = QK(g, 0); O(g - 1, 4); PV(g, SM(s0)); s1 = QK(g, 1); O(g - 1, 5); PV(g, SM(s1))
    s2 = QK(g, 2); O(g, 0, 'out'); PV(g, SM(s2)); s3 = QK(g, 3)
    O(g, 1, 'out'); O(g, 2, 'out'); PV(g, SM(s3)); O(g, 3, 'out'); O(g, 4, 'out'); O(g, 5, 'out')
    for j in range(NJ):
        out_cp(j).wait()


@jax.jit
def pallas_standalone__mha_block_cached__near_ridge_kernel(x, k_cache, v_cache, wq, wo):
    B, Sq, D = x.shape
    _, H, Sk, Dh = k_cache.shape
    M = B * Sq
    G = H // HG
    W = HG * Dh
    x2 = x.reshape(M, D)
    out = pl.pallas_call(
        functools.partial(_kernel, B=B, Sq=Sq, D=D, H=H, Dh=Dh, scale=Dh ** -0.5 * math.log2(math.e)),
        in_specs=[pl.BlockSpec(memory_space=pl.ANY)] * 5,
        out_specs=pl.BlockSpec(memory_space=pl.ANY),
        out_shape=jax.ShapeDtypeStruct((M, D), x.dtype),
        scratch_shapes=[
            pltpu.VMEM((M, D), bf16),
            pltpu.VMEM((G, B, HG, Sk, Dh), bf16),
            pltpu.VMEM((G, B, HG, Sk, Dh), bf16),
            pltpu.VMEM((G, D, W), bf16),
            pltpu.VMEM((G, D, W), bf16),
            pltpu.VMEM((D, M), f32),
            pltpu.VMEM((M, W), bf16),
            pltpu.VMEM((M, W), bf16),
            pltpu.VMEM((M, D), bf16),
            pltpu.VMEM((M, W), f32),
            pltpu.SemaphoreType.DMA((6,)),
        ],
        compiler_params=pltpu.CompilerParams(vmem_limit_bytes=96 * 1024 * 1024),
    )(x2, k_cache, v_cache, wq, wo.T)
    return out.reshape(B, Sq, D)
```

```python
import functools
import math
import jax
import jax.numpy as jnp
import jax.experimental.pallas as pl
import jax.experimental.pallas.tpu as pltpu

HG = 4
KA = 256
NT = (((1,), (1,)), ((), ()))
f32, bf16 = jnp.float32, jnp.bfloat16


def _kernel(x_hbm, k_hbm, v_hbm, wq_hbm, wot_hbm, o_hbm,
            x_v, k_v, v_v, wq_v, wot_v, acc_ref, q_ref, ob_ref, out_v, qp_ref, q0_ref, sems,
            *, B, Sq, D, H, Dh, scale):
    G = H // HG
    W = HG * Dh
    RP = 2 * Sq
    NJ = (B * Sq) // 128
    S1, S2, S3, S4, SL, SO = range(6)


    def wq_cp(g, s):
        return pltpu.make_async_copy(wq_hbm.at[:, pl.ds(g * W, W)], wq_v.at[g], sems.at[s])

    def wot_cp(g, s):
        return pltpu.make_async_copy(wot_hbm.at[:, pl.ds(g * W, W)], wot_v.at[g], sems.at[s])

    def k_cp(g, s):
        return pltpu.make_async_copy(k_hbm.at[:, pl.ds(g * HG, HG)], k_v.at[g], sems.at[s])

    def v_cp(g, s):
        return pltpu.make_async_copy(v_hbm.at[:, pl.ds(g * HG, HG)], v_v.at[g], sems.at[s])

    def out_cp(j):
        return pltpu.make_async_copy(out_v.at[pl.ds(j * 128, 128)], o_hbm.at[pl.ds(j * 128, 128)], sems.at[SO])

    def grp1():
        return (pltpu.make_async_copy(x_hbm.at[:, pl.ds(0, KA)], x_v.at[:, pl.ds(0, KA)], sems.at[S1]),
                pltpu.make_async_copy(wq_hbm.at[pl.ds(0, KA), pl.ds(0, W)], wq_v.at[0, pl.ds(0, KA)], sems.at[S1]))

    def grp2():
        return (pltpu.make_async_copy(x_hbm.at[:, pl.ds(KA, D - KA)], x_v.at[:, pl.ds(KA, D - KA)], sems.at[S2]),
                pltpu.make_async_copy(wq_hbm.at[pl.ds(KA, D - KA), pl.ds(0, W)], wq_v.at[0, pl.ds(KA, D - KA)],
                                      sems.at[S2]))

    def k0_cp(half, s):
        hb = B // 2
        return pltpu.make_async_copy(k_hbm.at[pl.ds(half * hb, hb), pl.ds(0, HG)], k_v.at[0, pl.ds(half * hb, hb)],
                                     sems.at[s])

    def grp3():
        return (wq_cp(1, S3), k0_cp(0, S3))

    def grp4():
        return (k0_cp(1, S4), v_cp(0, S4), wot_cp(0, S4))

    def kvo(g):
        return (k_cp(g, SL), v_cp(g, SL), wot_cp(g, SL))

    def start(cs, prio=1):
        for c in cs:
            c.start(priority=prio)

    def wait(cs):
        for c in cs:
            c.wait()

    def Q(g, bp):
        r = slice(bp * RP, (bp + 1) * RP)
        q_ref[r, :] = (jnp.dot(x_v[r, :], wq_v[g], preferred_element_type=f32) * scale).astype(bf16)

    def QK(g, bp, qr=q_ref):
        res = []
        for b in (2 * bp, 2 * bp + 1):
            for h in range(HG):
                qbh = qr[b * Sq:(b + 1) * Sq, h * Dh:(h + 1) * Dh]
                res.append((b, h, jax.lax.dot_general(qbh, k_v[g, b, h], NT, preferred_element_type=f32)))
        return res

    def SM(ss):
        res = []
        for b, h, s in ss:
            m = jnp.max(s, axis=-1, keepdims=True)
            p = jnp.exp2(s - m)
            l = jnp.sum(p, axis=-1, keepdims=True)
            r = pl.reciprocal(l, approx=True)
            r = r * (2.0 - l * r)
            res.append((b, h, p.astype(bf16), r))
        return res

    def PV(g, ps):
        for b, h, p, r in ps:
            o = jnp.dot(p, v_v[g, b, h], preferred_element_type=f32)
            ob_ref[b * Sq:(b + 1) * Sq, h * Dh:(h + 1) * Dh] = (o * r).astype(bf16)

    def O(g, j, mode='acc'):
        c = slice(j * 128, (j + 1) * 128)
        part = jax.lax.dot_general(wot_v[g], ob_ref[c, :], NT, preferred_element_type=f32)
        if mode == 'set':
            acc_ref[:, c] = part
        elif mode == 'out':
            out_v[c, :] = (acc_ref[:, c] + part).T.astype(out_v.dtype)
            out_cp(j).start()
        else:
            acc_ref[:, c] += part

    def ON(g, j):
        c = slice(j * 128, (j + 1) * 128)
        part = jax.lax.dot_general(ob_ref[c, :], wot_v[g], NT, preferred_element_type=f32)
        out_v[c, :] = (acc_ref[:, c].T + part).astype(out_v.dtype)
        out_cp(j).start()

    CS = 384

    def tail_cp(i):
        r = pl.ds((NJ - 1) * 128, 128)
        c = pl.ds(0, CS) if i == 0 else pl.ds(CS, D - CS)
        return pltpu.make_async_copy(out_v.at[r, c], o_hbm.at[r, c], sems.at[SO])

    def ONS(g, j):
        c = slice(j * 128, (j + 1) * 128)
        for i, n in enumerate((slice(0, CS), slice(CS, D))):
            part = jax.lax.dot_general(ob_ref[c, :], wot_v[g, n, :], NT, preferred_element_type=f32)
            out_v[c, n] = (acc_ref[n, c].T + part).astype(out_v.dtype)
            tail_cp(i).start()

    KT = (HG - 1) * Dh

    def OT(g, j):
        c = slice(j * 128, (j + 1) * 128)
        acc_ref[:, c] += jax.lax.dot_general(wot_v[g, :, :KT], ob_ref[c, :KT], NT, preferred_element_type=f32)

    def OL(g, j):
        c = slice(j * 128, (j + 1) * 128)
        part = jax.lax.dot_general(ob_ref[c, KT:], wot_v[g, :, KT:], NT, preferred_element_type=f32)
        out_v[c, :] = (acc_ref[:, c].T + part).astype(out_v.dtype)
        out_cp(j).start()

    start(grp1(), 0)
    start(grp2(), 1)
    acc_ref[:, 4 * 128:] = jnp.zeros((D, (NJ - 4) * 128), f32)
    wait(grp1())
    start(grp3())
    qp_ref[...] = jnp.dot(x_v[:, :KA], wq_v[0, :KA, :], preferred_element_type=f32)
    wait(grp2())
    start(grp4())
    q0_ref[...] = ((qp_ref[...] + jnp.dot(x_v[:, KA:], wq_v[0, KA:, :], preferred_element_type=f32)) * scale).astype(bf16)
    wait(grp3())
    start(kvo(1) + (wq_cp(2, SL),))
    Q(1, 0); s0 = QK(0, 0, q0_ref); Q(1, 1); p0 = SM(s0); s1 = QK(0, 1, q0_ref); Q(1, 2); p1 = SM(s1)
    wait(grp4())
    PV(0, p0); s2 = QK(0, 2, q0_ref); PV(0, p1); Q(1, 3); PV(0, SM(s2)); s3 = QK(0, 3, q0_ref); O(0, 0, 'set'); O(0, 1, 'set'); PV(0, SM(s3))
    O(0, 2, 'set'); O(0, 3, 'set')

    def body(g, carry):
        wait(kvo(g) + (wq_cp(g + 1, SL),))
        start(kvo(g + 1))

        @pl.when(g + 2 < G)
        def _():
            start((wq_cp(g + 2, SL),))

        s0 = QK(g, 0); O(g - 1, 4); PV(g, SM(s0)); s1 = QK(g, 1); O(g - 1, 5); Q(g + 1, 0); PV(g, SM(s1))
        s2 = QK(g, 2); O(g, 0); Q(g + 1, 1); PV(g, SM(s2)); s3 = QK(g, 3)
        O(g, 1); O(g, 2); Q(g + 1, 2); PV(g, SM(s3)); Q(g + 1, 3); O(g, 3)
        return carry

    jax.lax.fori_loop(1, G - 1, body, 0)

    g = G - 1
    wait(kvo(g))
    s0 = QK(g, 0); O(g - 1, 4); PV(g, SM(s0)); s1 = QK(g, 1); O(g - 1, 5); PV(g, SM(s1))
    s2 = QK(g, 2); OT(g, 0); PV(g, SM(s2)); s3 = QK(g, 3)
    OT(g, 1); OT(g, 2); OL(g, 0); PV(g, SM(s3)); OT(g, 3); OL(g, 1); OL(g, 2); ON(g, 4); OL(g, 3); ONS(g, 5)
    for j in range(NJ - 1):
        out_cp(j).wait()
    tail_cp(0).wait()
    tail_cp(1).wait()


@jax.jit
def pallas_standalone__mha_block_cached__near_ridge_kernel(x, k_cache, v_cache, wq, wo):
    B, Sq, D = x.shape
    _, H, Sk, Dh = k_cache.shape
    M = B * Sq
    G = H // HG
    W = HG * Dh
    x2 = x.reshape(M, D)
    out = pl.pallas_call(
        functools.partial(_kernel, B=B, Sq=Sq, D=D, H=H, Dh=Dh, scale=Dh ** -0.5 * math.log2(math.e)),
        in_specs=[pl.BlockSpec(memory_space=pl.ANY)] * 5,
        out_specs=pl.BlockSpec(memory_space=pl.ANY),
        out_shape=jax.ShapeDtypeStruct((M, D), x.dtype),
        scratch_shapes=[
            pltpu.VMEM((M, D), bf16),
            pltpu.VMEM((G, B, HG, Sk, Dh), bf16),
            pltpu.VMEM((G, B, HG, Sk, Dh), bf16),
            pltpu.VMEM((G, D, W), bf16),
            pltpu.VMEM((G, D, W), bf16),
            pltpu.VMEM((D, M), f32),
            pltpu.VMEM((M, W), bf16),
            pltpu.VMEM((M, W), bf16),
            pltpu.VMEM((M, D), bf16),
            pltpu.VMEM((M, W), f32),
            pltpu.VMEM((M, W), bf16),
            pltpu.SemaphoreType.DMA((6,)),
        ],
        compiler_params=pltpu.CompilerParams(vmem_limit_bytes=96 * 1024 * 1024, disable_bounds_checks=True,
                                             disable_semaphore_checks=True),
    )(x2, k_cache, v_cache, wq, wo.T)
    return out.reshape(B, Sq, D)
```

```python
import functools
import math

import jax
import jax.numpy as jnp
import jax.experimental.pallas as pl
import jax.experimental.pallas.tpu as pltpu

HG = 4
KA = 256
CS = 384
TJ = 128
NT = (((1,), (1,)), ((), ()))
f32, bf16 = jnp.float32, jnp.bfloat16


def _kernel(x_hbm, k_hbm, v_hbm, wq_hbm, wot_hbm, o_hbm,
            x_v, k_v, v_v, wq_v, wot_v, acc_ref, q_ref, ob_ref, out_v, qp_ref, q0_ref, sems,
            *, B, Sq, D, H, Dh, scale):
    G = H // HG
    W = HG * Dh
    RP = 2 * Sq
    NJ = (B * Sq) // TJ
    KT = (HG - 1) * Dh
    S1, S2, S3, S4, SL, SO = range(6)

    def wq_cp(g, s):
        return pltpu.make_async_copy(wq_hbm.at[:, pl.ds(g * W, W)], wq_v.at[g], sems.at[s])

    def wot_cp(g, s):
        return pltpu.make_async_copy(wot_hbm.at[:, pl.ds(g * W, W)], wot_v.at[g], sems.at[s])

    def k_cp(g, s):
        return pltpu.make_async_copy(k_hbm.at[:, pl.ds(g * HG, HG)], k_v.at[g], sems.at[s])

    def v_cp(g, s):
        return pltpu.make_async_copy(v_hbm.at[:, pl.ds(g * HG, HG)], v_v.at[g], sems.at[s])

    def k0_cp(half, s):
        hb = B // 2
        return pltpu.make_async_copy(k_hbm.at[pl.ds(half * hb, hb), pl.ds(0, HG)],
                                     k_v.at[0, pl.ds(half * hb, hb)], sems.at[s])

    def xw_cp(k0, k1, s):
        ks = pl.ds(k0, k1 - k0)
        return (pltpu.make_async_copy(x_hbm.at[:, ks], x_v.at[:, ks], sems.at[s]),
                pltpu.make_async_copy(wq_hbm.at[ks, pl.ds(0, W)], wq_v.at[0, ks], sems.at[s]))

    def grp1():
        return xw_cp(0, KA, S1)

    def grp2():
        return xw_cp(KA, D, S2)

    def grp3():
        return (wq_cp(1, S3), k0_cp(0, S3))

    def grp4():
        return (k0_cp(1, S4), v_cp(0, S4), wot_cp(0, S4))

    def kvo(g):
        return (k_cp(g, SL), v_cp(g, SL), wot_cp(g, SL))

    def out_cp(j):
        r = pl.ds(j * TJ, TJ)
        return pltpu.make_async_copy(out_v.at[r], o_hbm.at[r], sems.at[SO])

    def tail_cp(i):
        r = pl.ds((NJ - 1) * TJ, TJ)
        c = pl.ds(0, CS) if i == 0 else pl.ds(CS, D - CS)
        return pltpu.make_async_copy(out_v.at[r, c], o_hbm.at[r, c], sems.at[SO])

    def start(cs, prio=1):
        for c in cs:
            c.start(priority=prio)

    def wait(cs):
        for c in cs:
            c.wait()

    def dot_nt(a, b):
        return jax.lax.dot_general(a, b, NT, preferred_element_type=f32)

    def Q(g, bp):
        r = slice(bp * RP, (bp + 1) * RP)
        q_ref[r, :] = (jnp.dot(x_v[r, :], wq_v[g], preferred_element_type=f32) * scale).astype(bf16)

    def load_q(bp, qr):
        return [(b, h, qr[b * Sq:(b + 1) * Sq, h * Dh:(h + 1) * Dh])
                for b in (2 * bp, 2 * bp + 1) for h in range(HG)]

    def scores(g, qs):
        return [(b, h, dot_nt(qq, k_v[g, b, h])) for b, h, qq in qs]

    def QK(g, bp, qr=q_ref):
        return scores(g, load_q(bp, qr))

    def SM(ss):
        res = []
        for b, h, s in ss:
            m = jnp.max(s, axis=-1, keepdims=True)
            p = jnp.exp2(s - m)
            l = jnp.sum(p, axis=-1, keepdims=True)
            r = pl.reciprocal(l, approx=True)
            r = r * (2.0 - l * r)
            res.append((b, h, p.astype(bf16), r))
        return res

    def PV(g, ps):
        for b, h, p, r in ps:
            o = jnp.dot(p, v_v[g, b, h], preferred_element_type=f32)
            ob_ref[b * Sq:(b + 1) * Sq, h * Dh:(h + 1) * Dh] = (o * r).astype(bf16)

    def O(g, j, first=False):
        c = slice(j * TJ, (j + 1) * TJ)
        part = dot_nt(wot_v[g], ob_ref[c, :])
        if first:
            acc_ref[:, c] = part
        else:
            acc_ref[:, c] += part

    def OT(g, j):
        c = slice(j * TJ, (j + 1) * TJ)
        acc_ref[:, c] += dot_nt(wot_v[g, :, :KT], ob_ref[c, :KT])

    def OL(g, j):
        c = slice(j * TJ, (j + 1) * TJ)
        part = dot_nt(ob_ref[c, KT:], wot_v[g, :, KT:])
        out_v[c, :] = (acc_ref[:, c].T + part).astype(out_v.dtype)
        out_cp(j).start()

    def ON(g, j):
        c = slice(j * TJ, (j + 1) * TJ)
        part = dot_nt(ob_ref[c, :], wot_v[g])
        out_v[c, :] = (acc_ref[:, c].T + part).astype(out_v.dtype)
        out_cp(j).start()

    def ONS(g, j):
        c = slice(j * TJ, (j + 1) * TJ)
        for i, n in enumerate((slice(0, CS), slice(CS, D))):
            part = dot_nt(ob_ref[c, :], wot_v[g, n, :])
            out_v[c, n] = (acc_ref[n, c].T + part).astype(out_v.dtype)
            tail_cp(i).start()

    start(grp1(), 0)
    start(grp2(), 1)
    acc_ref[:, 4 * TJ:] = jnp.zeros((D, (NJ - 4) * TJ), f32)
    wait(grp1())
    start(grp3())
    qp_ref[...] = jnp.dot(x_v[:, :KA], wq_v[0, :KA, :], preferred_element_type=f32)
    wait(grp2())
    start(grp4())
    q0_ref[...] = ((qp_ref[...] + jnp.dot(x_v[:, KA:], wq_v[0, KA:, :], preferred_element_type=f32))
                   * scale).astype(bf16)
    wait(grp3())
    start(kvo(1) + (wq_cp(2, SL),))
    Q(1, 0); s0 = QK(0, 0, q0_ref); Q(1, 1); p0 = SM(s0); s1 = QK(0, 1, q0_ref); Q(1, 2); p1 = SM(s1)
    wait(grp4())
    PV(0, p0); s2 = QK(0, 2, q0_ref); PV(0, p1); Q(1, 3); PV(0, SM(s2)); s3 = QK(0, 3, q0_ref)
    O(0, 0, True); O(0, 1, True); PV(0, SM(s3)); O(0, 2, True); O(0, 3, True)

    def body(g, carry):
        wait(kvo(g) + (wq_cp(g + 1, SL),))
        qs = load_q(0, q_ref)
        Q(g + 1, 0)
        start(kvo(g + 1))

        @pl.when(g + 2 < G)
        def _():
            start((wq_cp(g + 2, SL),))

        s0 = scores(g, qs)
        O(g - 1, 4); PV(g, SM(s0)); s1 = QK(g, 1); O(g - 1, 5); PV(g, SM(s1))
        s2 = QK(g, 2); O(g, 0); Q(g + 1, 1); PV(g, SM(s2)); s3 = QK(g, 3)
        O(g, 1); O(g, 2); Q(g + 1, 2); PV(g, SM(s3)); Q(g + 1, 3); O(g, 3)
        return carry

    jax.lax.fori_loop(1, G - 1, body, 0)

    g = G - 1
    wait(kvo(g))
    s0 = QK(g, 0); O(g - 1, 4); PV(g, SM(s0)); s1 = QK(g, 1); O(g - 1, 5); PV(g, SM(s1))
    s2 = QK(g, 2); OT(g, 0); PV(g, SM(s2)); s3 = QK(g, 3)
    OT(g, 1); OT(g, 2); OL(g, 0); PV(g, SM(s3)); OT(g, 3); OL(g, 1); OL(g, 2); ON(g, 4); OL(g, 3); ONS(g, 5)
    for j in range(NJ - 1):
        out_cp(j).wait()
    tail_cp(0).wait()
    tail_cp(1).wait()


@jax.jit
def pallas_standalone__mha_block_cached__near_ridge_kernel(
    x: jax.Array,
    k_cache: jax.Array,
    v_cache: jax.Array,
    wq: jax.Array,
    wo: jax.Array,
):
    B, Sq, D = x.shape
    _, H, Sk, Dh = k_cache.shape
    assert (B, Sq, Sk, D, Dh) == (8, 96, 96, 576, 128) and H % HG == 0 and H // HG >= 3
    M = B * Sq
    G = H // HG
    W = HG * Dh
    out = pl.pallas_call(
        functools.partial(_kernel, B=B, Sq=Sq, D=D, H=H, Dh=Dh, scale=Dh ** -0.5 * math.log2(math.e)),
        in_specs=[pl.BlockSpec(memory_space=pl.ANY)] * 5,
        out_specs=pl.BlockSpec(memory_space=pl.ANY),
        out_shape=jax.ShapeDtypeStruct((M, D), x.dtype),
        scratch_shapes=[
            pltpu.VMEM((M, D), bf16),
            pltpu.VMEM((G, B, HG, Sk, Dh), bf16),
            pltpu.VMEM((G, B, HG, Sk, Dh), bf16),
            pltpu.VMEM((G, D, W), bf16),
            pltpu.VMEM((G, D, W), bf16),
            pltpu.VMEM((D, M), f32),
            pltpu.VMEM((M, W), bf16),
            pltpu.VMEM((M, W), bf16),
            pltpu.VMEM((M, D), bf16),
            pltpu.VMEM((M, W), f32),
            pltpu.VMEM((M, W), bf16),
            pltpu.SemaphoreType.DMA((6,)),
        ],
        compiler_params=pltpu.CompilerParams(
            vmem_limit_bytes=64 * 1024 * 1024,
            disable_bounds_checks=True,
            disable_semaphore_checks=True,
        ),
    )(x.reshape(M, D), k_cache, v_cache, wq, wo.T)
    return out.reshape(B, Sq, D)
```
